```python
import os as _os
_os.environ.setdefault("JAX_PLATFORMS", "cpu")
import jax
import jax.numpy as jnp

def _softmax(x, axis=-1):
    return jax.nn.softmax(x, axis=axis)
def _gelu(x):
    return jax.nn.gelu(x, approximate=True)
def _silu(x):
    return jax.nn.silu(x)
def _sigmoid(x):
    return jax.nn.sigmoid(x)
def _layernorm(x, axis=-1, eps=1e-5):
    m = jnp.mean(x, axis=axis, keepdims=True)
    v = jnp.var(x, axis=axis, keepdims=True)
    return (x - m) / jnp.sqrt(v + eps)
def _scatter_add(tgt, idx, src, axis=0):
    return tgt.at[idx].add(src)
def _segment_sum(src, seg, n):
    return jax.ops.segment_sum(src, seg, n)
class _Rng:
    def __init__(self, key):
        self._k = key
    def _next(self):
        self._k, sub = jax.random.split(self._k)
        return sub
    def normal(self, shape):
        return jax.random.normal(self._next(), shape, dtype=jnp.bfloat16)
    def randint(self, lo, hi, shape):
        return jax.random.randint(self._next(), shape, lo, hi, dtype=jnp.int32)
    def uniform(self, shape, lo=0.0, hi=1.0):
        return jax.random.uniform(self._next(), shape, jnp.bfloat16, lo, hi)
    def permutation(self, n):
        return jax.random.permutation(self._next(), n)


kernel_name = 'gated_mix__linear_attn_block__mixer_token_mlp__prompt'

def setup_inputs():
    _rng = _Rng(jax.random.key(int.from_bytes(__import__("os").urandom(4), "little")))
    _w = (lambda a: (lambda t: t.astype(jnp.bfloat16) if jnp.issubdtype(t.dtype, jnp.floating) else t)(jnp.asarray(a)))
    def _A_setup():
        B, S, D = 1, 2048, 512
        return {
            "x": _w((lambda *s: _rng.normal(s) * 0.05)(B, S, D)),
            "wqkv": _w((lambda *s: _rng.normal(s) * 0.8)(D, 3 * D)),
            "wo": _w((lambda *s: _rng.normal(s) * 0.05)(D, D)),
        }
    _A_in = _A_setup()

    def _B_setup():
        B, S, D, F = 1, 2048, 512, 1792
        return {
            "x": _w((lambda *s: _rng.normal(s) * 0.05)(B, S, D)),
            "w1": _w((lambda *s: _rng.normal(s) * 0.1)(S, F) * (S ** -0.5)),
            "b1": _w((lambda *s: _rng.normal(s) * 0.1)(F) * 0.02),
            "w2": _w((lambda *s: _rng.normal(s) * 0.1)(F, S) * (F ** -0.5)),
            "b2": _w((lambda *s: _rng.normal(s) * 0.1)(S) * 0.02),
        }
    _B_in = _B_setup()

    return {
        "A_x": _A_in["x"],
        "A_wqkv": _A_in["wqkv"],
        "A_wo": _A_in["wo"],
        "B_x": _B_in["x"],
        "B_w1": _B_in["w1"],
        "B_b1": _B_in["b1"],
        "B_w2": _B_in["w2"],
        "B_b2": _B_in["b2"],
        "gate_w": _w((lambda *s: _rng.normal(s) * 0.05)(512) * 16.0),
    }

def reference(A_x, A_wqkv, A_wo, B_x, B_w1, B_b1, B_w2, B_b2, gate_w):
    def _A_ref(x, wqkv, wo):
        B, S, D = x.shape
        H = 32; Dh = D // H
        qkv = (lambda x, *d: x.transpose(*d))((x @ wqkv).reshape(B, S, 3, H, Dh), 2, 0, 3, 1, 4)
        q, k, v = qkv[0], qkv[1], qkv[2]
        phi = lambda t: jnp.where(t > 0, t + 1, jnp.exp(t)) + 1e-6
        pq, pk = phi(q), phi(k)
        kv = jnp.einsum("bhsd,bhse->bhde", pk, v)
        z = jnp.einsum("bhsd->bhd", pk)
        num = jnp.einsum("bhqd,bhde->bhqe", pq, kv)
        den = jnp.einsum("bhqd,bhd->bhq", pq, z)[..., None] + 1e-6
        o = num / den
        return (lambda x, *d: x.transpose(*d))(o, 0, 2, 1, 3).reshape(B, S, D) @ wo

    def _B_ref(x, w1, b1, w2, b2):
        B, S, D = x.shape
        h = _layernorm(x, axis=-1)
        u = jnp.einsum("bsd,sf->bdf", h, w1) + b1
        u = _gelu(u)
        y = jnp.einsum("bdf,fs->bds", u, w2) + b2
        return (lambda x, *d: x.transpose(*d))(y, 0, 2, 1)

    x = A_x
    g = _sigmoid((x * gate_w).sum(-1, keepdims=True))
    a = _A_ref(x, A_wqkv, A_wo)
    b = _B_ref(x, B_w1, B_b1, B_w2, B_b2)
    return g * a + (1 - g) * b
```

```python
import math

import jax
import jax.numpy as jnp
import jax.experimental.pallas as pl
import jax.experimental.pallas.tpu as pltpu

_H = 32
_SQRT_2_OVER_PI = math.sqrt(2.0 / math.pi)
_G = 128
_XC = 512
_TF = 256
_TS = 512


def _phi(t):
    return jnp.where(t > 0, t + 1.0, jnp.exp(t)) + 1e-6


def _gelu_tanh(u):
    return 0.5 * u * (1.0 + jnp.tanh(_SQRT_2_OVER_PI * (u + 0.044715 * (u * u * u))))


def _kernel(x_hbm, wqkv_hbm, wo_hbm, w1_hbm, b1_ref, w2_hbm, b2_ref, gw_ref, out_hbm,
            x_v, wqkv_v, wo_v, w1_v, w2_v, xT_v, hT_v, v_v, gu_v, m2_v, zb_v, a_v, obuf,
            xsems, sems, osems):
    S, D = x_v.shape
    F = w1_v.shape[1]
    Dh = D // _H
    bf16 = jnp.bfloat16
    f32 = jnp.float32
    NG = D // _G
    NXC = S // _XC

    def xcopy(c):
        return pltpu.make_async_copy(x_hbm.at[pl.ds(c * _XC, _XC), :],
                                     x_v.at[pl.ds(c * _XC, _XC), :], xsems.at[c])

    def wcopy(j):
        return pltpu.make_async_copy(wqkv_hbm.at[:, pl.ds(j * D, D)],
                                     wqkv_v.at[:, pl.ds(j * D, D)], sems.at[j])

    x_copies = [xcopy(c) for c in range(NXC)]
    cp_wq, cp_wk, cp_wv = wcopy(0), wcopy(1), wcopy(2)
    cp_w1 = pltpu.make_async_copy(w1_hbm, w1_v, sems.at[3])
    cp_wo = pltpu.make_async_copy(wo_hbm, wo_v, sems.at[4])
    cp_w2 = pltpu.make_async_copy(w2_hbm, w2_v, sems.at[5])
    x_copies[0].start()
    cp_wv.start()

    zcol = jnp.zeros((D, 1), f32)
    for c in range(NXC):
        sl = slice(c * _XC, (c + 1) * _XC)
        if c == 0:
            x_copies[0].wait()
            cp_wk.start()
            x_copies[1].start()
        elif c == 2:
            for cc in range(2, NXC):
                x_copies[cc].wait()
            cp_wq.wait()
            cp_wo.wait()
            cp_w1.start()
        xc = x_v[sl, :]
        xT = xc.T
        xTf = xT.astype(f32)
        mean = jnp.mean(xTf, axis=0, keepdims=True)
        cen = xTf - mean
        var = jnp.mean(cen * cen, axis=0, keepdims=True)
        hT_v[:, sl] = (cen / jnp.sqrt(var + 1e-5)).astype(bf16)
        if c == 0:
            cp_wv.wait()
        v_v[sl, :] = jnp.dot(xc, wqkv_v[:, 2 * D:3 * D], preferred_element_type=f32).astype(bf16)
        if c == 0:
            cp_wk.wait()
            x_copies[1].wait()
            for cc in range(2, NXC):
                x_copies[cc].start()
            cp_wq.start()
            cp_wo.start()
        kT = jax.lax.dot_general(wqkv_v[:, D:2 * D], xT, (((0,), (0,)), ((), ())),
                                 preferred_element_type=f32)
        pkT = _phi(kT)
        zcol = zcol + jnp.sum(pkT, axis=1, keepdims=True)
        xT_v[:, sl] = pkT.astype(bf16)

    ri = jax.lax.broadcasted_iota(jnp.int32, (_G, _G), 0) // Dh
    ci = jax.lax.broadcasted_iota(jnp.int32, (_G, _G), 1) // Dh
    same = ri == ci
    for g in range(NG):
        sl = slice(g * _G, (g + 1) * _G)
        kvg = jnp.dot(xT_v[sl, :], v_v[:, sl], preferred_element_type=f32)
        kvg = jnp.where(same, kvg, 0.0).astype(bf16)
        m2_v[sl, :] = jnp.dot(kvg, wo_v[sl, :], preferred_element_type=f32).astype(bf16)
        zb_v[sl, :] = jnp.where(same, jnp.broadcast_to(zcol[sl, :], (_G, _G)), 0.0).astype(bf16)

    def mixer1_tile(f):
        sl = slice(f * _TF, (f + 1) * _TF)
        u = jnp.dot(hT_v[...], w1_v[:, sl], preferred_element_type=f32)
        u = u + b1_ref[sl].astype(f32).reshape(1, _TF)
        gu_v[:, sl] = _gelu_tanh(u).astype(bf16)

    pq = _phi(jnp.dot(x_v[...], wqkv_v[:, 0:D], preferred_element_type=f32))
    pqb = pq.astype(bf16)
    cp_w1.wait()
    cp_w2.start()
    mixer1_tile(0)
    dens = []
    for g in range(NG):
        gs = slice(g * _G, (g + 1) * _G)
        dens.append(jnp.dot(pqb[:, gs], zb_v[gs, :], preferred_element_type=f32))
    den = jnp.concatenate(dens, axis=1) + 1e-6
    mixer1_tile(1)
    pqn = (pq / den).astype(bf16)
    mixer1_tile(2)
    a_v[...] = jnp.dot(pqn, m2_v[...], preferred_element_type=f32)
    for f in range(3, F // _TF):
        mixer1_tile(f)

    cp_w2.wait()
    gw = gw_ref[...].astype(f32).reshape(1, D)
    bounds = [0, 512, 1024, 1536, 1792, 2048]
    n_t = len(bounds) - 1
    out_copies = []
    for t in range(n_t):
        sl = slice(bounds[t], bounds[t + 1])
        ts = bounds[t + 1] - bounds[t]
        slot = t
        y = jnp.dot(gu_v[...], w2_v[:, sl], preferred_element_type=f32) + b2_ref[sl].astype(f32).reshape(1, ts)
        gate = jax.nn.sigmoid(jnp.sum(x_v[sl, :].astype(f32) * gw, axis=-1, keepdims=True))
        obuf[slot, 0:ts, :] = (gate * a_v[sl, :] + (1.0 - gate) * y.T).astype(obuf.dtype)
        cp = pltpu.make_async_copy(obuf.at[slot, pl.ds(0, ts), :], out_hbm.at[pl.ds(bounds[t], ts), :], osems.at[t])
        cp.start()
        out_copies.append(cp)
    for t in range(n_t):
        out_copies[t].wait()


@jax.jit
def pallas_gated_mix__linear_attn_block__mixer_token_mlp__prompt_kernel(
    A_x: jax.Array,
    A_wqkv: jax.Array,
    A_wo: jax.Array,
    B_x: jax.Array,
    B_w1: jax.Array,
    B_b1: jax.Array,
    B_w2: jax.Array,
    B_b2: jax.Array,
    gate_w: jax.Array,
):
    B, S, D = A_x.shape
    F = B_w1.shape[1]
    x2 = A_x.reshape(S, D)
    bf16 = jnp.bfloat16
    any_spec = pl.BlockSpec(memory_space=pl.ANY)
    vmem_spec = pl.BlockSpec(memory_space=pltpu.VMEM)
    out = pl.pallas_call(
        _kernel,
        out_shape=jax.ShapeDtypeStruct((S, D), A_x.dtype),
        in_specs=[any_spec, any_spec, any_spec, any_spec, vmem_spec, any_spec, vmem_spec, vmem_spec],
        out_specs=any_spec,
        scratch_shapes=[
            pltpu.VMEM((S, D), bf16),
            pltpu.VMEM((D, 3 * D), bf16),
            pltpu.VMEM((D, D), bf16),
            pltpu.VMEM((S, F), bf16),
            pltpu.VMEM((F, S), bf16),
            pltpu.VMEM((D, S), bf16),
            pltpu.VMEM((D, S), bf16),
            pltpu.VMEM((S, D), bf16),
            pltpu.VMEM((D, F), bf16),
            pltpu.VMEM((D, D), bf16),
            pltpu.VMEM((D, _G), bf16),
            pltpu.VMEM((S, D), jnp.float32),
            pltpu.VMEM((5, _TS, D), bf16),
            pltpu.SemaphoreType.DMA((S // _XC,)),
            pltpu.SemaphoreType.DMA((6,)),
            pltpu.SemaphoreType.DMA((5,)),
        ],
        compiler_params=pltpu.CompilerParams(vmem_limit_bytes=100 * 1024 * 1024),
    )(x2, A_wqkv, A_wo, B_w1, B_b1, B_w2, B_b2, gate_w)
    return out.reshape(B, S, D)
```

```python
import math

import jax
import jax.numpy as jnp
import jax.experimental.pallas as pl
import jax.experimental.pallas.tpu as pltpu

_H = 32
_SQRT_2_OVER_PI = math.sqrt(2.0 / math.pi)
_G = 128
_XBOUNDS = (0, 512, 1024, 1536, 2048)
_TF = 256
_TS = 512


def _phi(t):
    return jnp.where(t > 0, t + 1.0, jnp.exp(t)) + 1e-6


def _gelu_tanh(u):
    return 0.5 * u * (1.0 + jnp.tanh(_SQRT_2_OVER_PI * (u + 0.044715 * (u * u * u))))


def _kernel(x_hbm, wqkv_hbm, wo_hbm, w1_hbm, b1_hbm, w2_hbm, b2_hbm, gw_hbm, out_hbm,
            b1_ref, b2_ref, gw_ref, x_v, wqkv_v, wo_v, w1_v, w2_v, xT_v, hT_v, v_v, gu_v, m2_v, zb_v, a_v, obuf,
            xsems, sems, osems):
    S, D = x_v.shape
    F = w1_v.shape[1]
    Dh = D // _H
    bf16 = jnp.bfloat16
    f32 = jnp.float32
    NG = D // _G
    xb = _XBOUNDS
    NXC = len(xb) - 1

    def xcopy(c):
        return pltpu.make_async_copy(x_hbm.at[pl.ds(xb[c], xb[c + 1] - xb[c]), :],
                                     x_v.at[pl.ds(xb[c], xb[c + 1] - xb[c]), :], xsems.at[c])

    def wcopy(j):
        return pltpu.make_async_copy(wqkv_hbm.at[:, pl.ds(j * D, D)],
                                     wqkv_v.at[:, pl.ds(j * D, D)], sems.at[j])

    x_copies = [xcopy(c) for c in range(NXC)]
    cp_wq, cp_wk, cp_wv = wcopy(0), wcopy(1), wcopy(2)
    cp_w1 = pltpu.make_async_copy(w1_hbm, w1_v, sems.at[3])
    cp_wo = pltpu.make_async_copy(wo_hbm, wo_v, sems.at[4])
    cp_w2 = pltpu.make_async_copy(w2_hbm, w2_v, sems.at[5])
    cp_small = [pltpu.make_async_copy(b1_hbm, b1_ref, sems.at[6]),
                pltpu.make_async_copy(b2_hbm, b2_ref, sems.at[7]),
                pltpu.make_async_copy(gw_hbm, gw_ref, sems.at[8])]
    x_copies[0].start()
    cp_wv.start()
    for cp in cp_small:
        cp.start()

    zcol = jnp.zeros((D, 1), f32)
    for c in range(NXC):
        sl = slice(xb[c], xb[c + 1])
        if c == 0:
            x_copies[0].wait()
            cp_wk.start()
            x_copies[1].start()
        elif c == 2:
            for cc in range(2, NXC):
                x_copies[cc].wait()
            cp_wq.wait()
            cp_wo.wait()
            for cp in cp_small:
                cp.wait()
            cp_w1.start()
        xc = x_v[sl, :]
        xT = xc.T
        xTf = xT.astype(f32)
        mean = jnp.mean(xTf, axis=0, keepdims=True)
        cen = xTf - mean
        var = jnp.mean(cen * cen, axis=0, keepdims=True)
        hT_v[:, sl] = (cen * jax.lax.rsqrt(var + 1e-5)).astype(bf16)
        if c == 0:
            cp_wv.wait()
        v_v[sl, :] = jnp.dot(xc, wqkv_v[:, 2 * D:3 * D], preferred_element_type=f32).astype(bf16)
        if c == 0:
            cp_wk.wait()
            x_copies[1].wait()
            for cc in range(2, NXC):
                x_copies[cc].start()
            cp_wq.start()
            cp_wo.start()
        kT = jax.lax.dot_general(wqkv_v[:, D:2 * D], xT, (((0,), (0,)), ((), ())),
                                 preferred_element_type=f32)
        pkT = _phi(kT)
        zcol = zcol + jnp.sum(pkT, axis=1, keepdims=True)
        xT_v[:, sl] = pkT.astype(bf16)

    ri = jax.lax.broadcasted_iota(jnp.int32, (_G, _G), 0) // Dh
    ci = jax.lax.broadcasted_iota(jnp.int32, (_G, _G), 1) // Dh
    same = ri == ci
    for g in range(NG):
        sl = slice(g * _G, (g + 1) * _G)
        kvg = jnp.dot(xT_v[sl, :], v_v[:, sl], preferred_element_type=f32)
        kvg = jnp.where(same, kvg, 0.0).astype(bf16)
        m2_v[sl, :] = jnp.dot(kvg, wo_v[sl, :], preferred_element_type=f32).astype(bf16)
        zb_v[sl, :] = jnp.where(same, jnp.broadcast_to(zcol[sl, :], (_G, _G)), 0.0).astype(bf16)

    def mixer1_tile(f):
        sl = slice(f * _TF, (f + 1) * _TF)
        u = jnp.dot(hT_v[...], w1_v[:, sl], preferred_element_type=f32)
        u = u + b1_ref[sl].astype(f32).reshape(1, _TF)
        gu_v[:, sl] = _gelu_tanh(u).astype(bf16)

    pq = _phi(jnp.dot(x_v[...], wqkv_v[:, 0:D], preferred_element_type=f32))
    pqb = pq.astype(bf16)
    cp_w1.wait()
    cp_w2.start()
    mixer1_tile(0)
    dens = []
    for g in range(NG):
        gs = slice(g * _G, (g + 1) * _G)
        dens.append(jnp.dot(pqb[:, gs], zb_v[gs, :], preferred_element_type=f32))
    den = jnp.concatenate(dens, axis=1) + 1e-6
    mixer1_tile(1)
    r0 = pl.reciprocal(den, approx=True)
    rden = r0 * (2.0 - den * r0)
    pqn = (pq * rden).astype(bf16)
    mixer1_tile(2)
    a_v[...] = jnp.dot(pqn, m2_v[...], preferred_element_type=f32)
    for f in range(3, F // _TF):
        mixer1_tile(f)

    cp_w2.wait()
    gw = gw_ref[...].astype(f32).reshape(1, D)
    bounds = [0, 512, 1024, 1536, 1792, 1920, 2048]
    n_t = len(bounds) - 1
    out_copies = []
    for t in range(n_t):
        sl = slice(bounds[t], bounds[t + 1])
        ts = bounds[t + 1] - bounds[t]
        slot = t
        y = jnp.dot(gu_v[...], w2_v[:, sl], preferred_element_type=f32) + b2_ref[sl].astype(f32).reshape(1, ts)
        gate = jax.nn.sigmoid(jnp.sum(x_v[sl, :].astype(f32) * gw, axis=-1, keepdims=True))
        obuf[slot, 0:ts, :] = (gate * a_v[sl, :] + (1.0 - gate) * y.T).astype(obuf.dtype)
        cp = pltpu.make_async_copy(obuf.at[slot, pl.ds(0, ts), :], out_hbm.at[pl.ds(bounds[t], ts), :], osems.at[t])
        cp.start()
        out_copies.append(cp)
    for t in range(n_t):
        out_copies[t].wait()


@jax.jit
def pallas_gated_mix__linear_attn_block__mixer_token_mlp__prompt_kernel(
    A_x: jax.Array,
    A_wqkv: jax.Array,
    A_wo: jax.Array,
    B_x: jax.Array,
    B_w1: jax.Array,
    B_b1: jax.Array,
    B_w2: jax.Array,
    B_b2: jax.Array,
    gate_w: jax.Array,
):
    B, S, D = A_x.shape
    F = B_w1.shape[1]
    x2 = A_x.reshape(S, D)
    bf16 = jnp.bfloat16
    any_spec = pl.BlockSpec(memory_space=pl.ANY)
    vmem_spec = pl.BlockSpec(memory_space=pltpu.VMEM)
    out = pl.pallas_call(
        _kernel,
        out_shape=jax.ShapeDtypeStruct((S, D), A_x.dtype),
        in_specs=[any_spec] * 8,
        out_specs=any_spec,
        scratch_shapes=[
            pltpu.VMEM((F,), bf16),
            pltpu.VMEM((S,), bf16),
            pltpu.VMEM((D,), bf16),
            pltpu.VMEM((S, D), bf16),
            pltpu.VMEM((D, 3 * D), bf16),
            pltpu.VMEM((D, D), bf16),
            pltpu.VMEM((S, F), bf16),
            pltpu.VMEM((F, S), bf16),
            pltpu.VMEM((D, S), bf16),
            pltpu.VMEM((D, S), bf16),
            pltpu.VMEM((S, D), bf16),
            pltpu.VMEM((D, F), bf16),
            pltpu.VMEM((D, D), bf16),
            pltpu.VMEM((D, _G), bf16),
            pltpu.VMEM((S, D), jnp.float32),
            pltpu.VMEM((6, _TS, D), bf16),
            pltpu.SemaphoreType.DMA((len(_XBOUNDS) - 1,)),
            pltpu.SemaphoreType.DMA((9,)),
            pltpu.SemaphoreType.DMA((6,)),
        ],
        compiler_params=pltpu.CompilerParams(vmem_limit_bytes=100 * 1024 * 1024),
    )(x2, A_wqkv, A_wo, B_w1, B_b1, B_w2, B_b2, gate_w)
    return out.reshape(B, S, D)
```
